```python
import jax
import jax.numpy as jnp

def _softmax(x, axis=-1):
    return jax.nn.softmax(x, axis=axis)
def _gelu(x):
    return jax.nn.gelu(x, approximate=True)
def _silu(x):
    return jax.nn.silu(x)
def _sigmoid(x):
    return jax.nn.sigmoid(x)
def _layernorm(x, axis=-1, eps=1e-5):
    m = jnp.mean(x, axis=axis, keepdims=True)
    v = jnp.var(x, axis=axis, keepdims=True)
    return (x - m) / jnp.sqrt(v + eps)
def _scatter_add(tgt, idx, src, axis=0):
    return tgt.at[idx].add(src)
def _segment_sum(src, seg, n):
    return jax.ops.segment_sum(src, seg, n)
class _Rng:
    def __init__(self, key):
        self._k = key
    def _next(self):
        self._k, sub = jax.random.split(self._k)
        return sub
    def normal(self, shape):
        return jax.random.normal(self._next(), shape, dtype=jnp.bfloat16)
    def randint(self, lo, hi, shape):
        return jax.random.randint(self._next(), shape, lo, hi, dtype=jnp.int32)
    def uniform(self, shape, lo=0.0, hi=1.0):
        return jax.random.uniform(self._next(), shape, jnp.bfloat16, lo, hi)
    def permutation(self, n):
        return jax.random.permutation(self._next(), n)


kernel_name = 'standalone__mha_softmax__near_ridge'

def _fwd_setup_inputs():
    _rng = _Rng(jax.random.key(int.from_bytes(__import__("os").urandom(4), "little")))
    _w = (lambda a: (lambda t: t.astype(jnp.bfloat16) if jnp.issubdtype(t.dtype, jnp.floating) else t)(jnp.asarray(a)))
    B, H, Sq, Sk, D = 16, 32, 384, 1024, 128
    return {
        "q": _w((lambda *s: _rng.normal(s) * 0.05)(B, H, Sq, D)),
        "k": _w((lambda *s: _rng.normal(s) * 0.05)(B, H, Sk, D)),
        "v": _w((lambda *s: _rng.normal(s) * 0.05)(B, H, Sk, D)),
    }

def _fwd_reference(q, k, v):
    scale = q.shape[-1] ** -0.5
    scores = jnp.einsum("bhqd,bhkd->bhqk", q, k) * scale
    p = _softmax(scores, axis=-1)
    return jnp.einsum("bhqk,bhkd->bhqd", p, v)


def setup_inputs():
    _inp = _fwd_setup_inputs()
    _gk = jax.random.fold_in(jax.random.key(int.from_bytes(__import__("os").urandom(4), "little")), 2**31 - 1)
    _shapes = [[16, 32, 384, 128]]
    _dtypes = ['bfloat16']
    _gks = jax.random.split(_gk, len(_shapes))
    _gs = [jax.random.normal(k, s, dtype=jnp.dtype(d)) * 0.05 for k, s, d in zip(_gks, _shapes, _dtypes)]
    _inp["grad_out"] = _gs[0]
    return _inp

def reference(q, k, v, grad_out):
    _const = dict()
    def _f(*_d):
        return _fwd_reference(**{'q': _d[0], 'k': _d[1], 'v': _d[2], **_const})
    _out, _vjp = jax.vjp(_f, q, k, v)
    _grads = _vjp(grad_out)
    _out0 = jnp.asarray(_out)
    return (_out0, *[jnp.asarray(_g) for _g in _grads])
```

```python
import jax, jax.numpy as jnp, functools
from jax import lax
import jax.experimental.pallas as pl
import jax.experimental.pallas.tpu as pltpu
NT = (((1,), (1,)), ((), ())); NN = (((1,), (0,)), ((), ())); TN = (((0,), (0,)), ((), ()))
f32 = jnp.float32; bf16 = jnp.bfloat16
def dot(a, b, dn): return lax.dot_general(a, b, dn, preferred_element_type=f32)
scale = 128 ** -0.5
C = scale * 1.4426950408889634

class Head:
    def __init__(s, h, refs, qb, kc, pf32):
        s.h = h; s.qb = qb; s.kc = kc; s.pf32 = pf32; s.nq = 384 // qb
        s.q, s.k, s.v, s.do, s.o, s.dq, s.dk, s.dv = refs
        s.P, s.PB, s.R, s.DELTA, s.DOV, s.DOS, s.DS = {}, {}, {}, {}, {}, {}, {}
    def rows(s, a): return slice(a * s.qb, (a + 1) * s.qb)
    def S(s, a):
        x = dot(s.q[s.h, s.rows(a), :], s.k[s.h], NT)
        m = jnp.max(x, axis=1, keepdims=True)
        p = jnp.exp2((x - m) * C)
        l = jnp.sum(p, axis=1, keepdims=True)
        s.R[a] = 1.0 / l
        s.PB[a] = p.astype(bf16); s.P[a] = p
    def O(s, a):
        o = dot(s.PB[a], s.v[s.h], NN) * s.R[a]
        s.o[s.h, s.rows(a), :] = o.astype(bf16)
        dof = s.do[s.h, s.rows(a), :].astype(f32) * s.R[a]
        s.DOV[a] = dof.astype(bf16); dos = dof * scale; s.DOS[a] = dos.astype(bf16)
        s.DELTA[a] = jnp.sum(dos * o, axis=1, keepdims=True)
    def D(s, a):
        dp = dot(s.DOS[a], s.v[s.h], NT)
        p = s.P[a] if s.pf32 else s.PB[a].astype(f32)
        s.DS[a] = (p * (dp - s.DELTA[a])).astype(bf16)
    def Q(s, a):
        s.dq[s.h, s.rows(a), :] = dot(s.DS[a], s.k[s.h], NN).astype(bf16)
    def T(s, X, W, ref, c):
        cs = slice(c * s.kc, (c + 1) * s.kc)
        acc = None
        for a in range(s.nq):
            t = dot(X[a][:, cs], W(a), TN)
            acc = t if acc is None else acc + t
        ref[s.h, cs, :] = acc.astype(bf16)
    def run(s, st):
        if st == "V":
            for c in range(1024 // s.kc): s.T(s.PB, lambda a: s.DOV[a], s.dv, c)
        elif st == "K":
            for c in range(1024 // s.kc): s.T(s.DS, lambda a: s.q[s.h, s.rows(a), :], s.dk, c)
        else:
            for a in range(s.nq): dict(S=s.S, O=s.O, D=s.D, Q=s.Q)[st](a)

def make(qb=128, kc=256, pf32=False, order="ODVsQK", hb=4):
    def body(*refs):
        hs = [Head(h, refs, qb, kc, pf32) for h in range(hb)]
        hs[0].run("S")
        for h in range(hb):
            for st in order:
                if st == "s":
                    if h + 1 < hb: hs[h + 1].run("S")
                else: hs[h].run(st)
    @jax.jit
    def mha(q, k, v, grad_out):
        do = grad_out
        B, H, Sq, D = q.shape; Sk = k.shape[2]
        r = lambda x: x.reshape(B * H, x.shape[2], D)
        sq = pl.BlockSpec((hb, Sq, D), lambda i: (i, 0, 0)); sk = pl.BlockSpec((hb, Sk, D), lambda i: (i, 0, 0))
        oq = jax.ShapeDtypeStruct((B * H, Sq, D), bf16); ok = jax.ShapeDtypeStruct((B * H, Sk, D), bf16)
        outs = pl.pallas_call(body, grid=(B * H // hb,), in_specs=[sq, sk, sk, sq], out_specs=[sq, sq, sk, sk],
            out_shape=[oq, oq, ok, ok], name="mha_k2",
            compiler_params=pltpu.CompilerParams(dimension_semantics=("arbitrary",), vmem_limit_bytes=100 * 2**20),
        )(r(q), r(k), r(v), r(do))
        return tuple(o.reshape(B, H, o.shape[1], D) for o in outs)
    return mha

pallas_standalone__mha_softmax__near_ridge_kernel = make()
```

```python
import jax
import jax.numpy as jnp
from jax import lax
import jax.experimental.pallas as pl
import jax.experimental.pallas.tpu as pltpu

F32, BF16, U32 = jnp.float32, jnp.bfloat16, jnp.uint32
NT, NN, TN = (((1,), (1,)), ((), ())), (((1,), (0,)), ((), ())), (((0,), (0,)), ((), ()))
SQ, SK, D, NH = 384, 1024, 128, 512
QB, KC = 128, 256
HB, R = 14, 8
NSTEPS = (NH - R) // HB
GROUPS = (8, 11, 13, 14)
SCALE = D ** -0.5
EXP2_SCALE = SCALE * 1.4426950408889634
IOFF, ILEN = (0, 384, 1408, 2432), (SQ, SK, SK, SQ)
OOFF, OLEN = (0, 2432, 1408, 384), (SQ, SQ, SK, SK)
ROWS = 2 * (SQ + SK)
OUT = {"O": 0, "Q": 1, "K": 2, "V": 3}
PRE = "Q0 s0 s1"
FIRST = "O0 S2 O1 D0 O2 D1 D2 V0 V1 V2 K0 K1 K2 s0 Q0 s1 Q1 s2 Q2"
MID = "O0 D0 O1 D1 O2 D2 V0 V1 V2 K0 K1 K2 s0 Q0 s1 Q1 s2 Q2"
LAST = "O0 D0 O1 D1 O2 D2 V0 V1 V2 K0 K1 K2 C0 Q1 Q2"
RAMP = "O0 S2 O1 D0 O2 D1 D2 V0 V1 V2 K0 K1 K2 C0 Q1 Q2"


def _dot(a, b, dn):
    return lax.dot_general(a, b, dn, preferred_element_type=F32)


def _rows(a):
    return slice(a * QB, (a + 1) * QB)


def _put(ref, a, x):
    ref[a * 64:(a + 1) * 64, :] = pltpu.bitcast(x, U32)


def _get(ref, a, cols=slice(None)):
    return pltpu.bitcast(ref[a * 64:(a + 1) * 64, cols], BF16)


def _load(ref, a=None):
    r = ref.bitcast(U32)
    return pltpu.bitcast(r[...] if a is None else r[a * 64:(a + 1) * 64, :], BF16)


class _Head:
    def __init__(self, refs, pb, ds, kc, dsc=None):
        self.q, self.k, self.v, self.do, self.o, self.dq, self.dk, self.dv = refs
        self.pb, self.ds, self.kc, self.dsc = pb, ds, kc, dsc
        self.l, self.delta, self.dov, self.dos, self.acc = {}, {}, {}, {}, {}

    def run(self, stage, a, chain):
        if stage == "S":
            x = _dot(_load(self.q, a), _load(self.k), NT)
            m = jnp.max(x, axis=1, keepdims=True)
            if chain:
                m = jnp.where(chain[-1] < 0, 0.0, m)
            p = jnp.exp2((x - m) * EXP2_SCALE)
            self.l[a] = jnp.sum(p, axis=1, keepdims=True)
            chain.append(self.l[a])
            _put(self.pb, a, p.astype(BF16))
        elif stage == "O":
            l = self.l[a]
            r0 = pl.reciprocal(l, approx=True)
            r = r0 * (2.0 - l * r0)
            o = _dot(_get(self.pb, a), _load(self.v), NN) * r
            self.o[_rows(a), :] = o.astype(BF16)
            dof = self.do[_rows(a), :].astype(F32) * r
            self.dov[a] = dof.astype(BF16)
            dos = dof * SCALE
            self.dos[a] = dos.astype(BF16)
            self.delta[a] = jnp.sum(dos * o, axis=1, keepdims=True)
        elif stage == "D":
            dp = _dot(self.dos[a], _load(self.v), NT)
            d = (_get(self.pb, a).astype(F32) * (dp - self.delta[a])).astype(BF16)
            _put(self.ds, a, d)
            if self.dsc is not None and a == 0:
                _put(self.dsc, a, d)
        elif stage == "Q":
            d = _get(self.ds, a)
            k = pltpu.bitcast(self.kc[...], BF16) if self.k is None else _load(self.k)
            self.dq[_rows(a), :] = _dot(d, k, NN).astype(BF16)
        elif stage == "C":
            self.kc[...] = self.k.bitcast(U32)[...]
        else:
            for n in range(4 * a, 4 * a + 4):
                c, b = divmod(n, 3)
                cols = slice(c * KC, (c + 1) * KC)
                if stage == "V":
                    t = _dot(_get(self.pb, b, cols), self.dov[b], TN)
                else:
                    t = _dot(_get(self.ds, b, cols), _load(self.q, b), TN)
                self.acc[stage] = t if b == 0 else self.acc[stage] + t
                if b == 2:
                    (self.dv if stage == "V" else self.dk)[cols, :] = self.acc[stage].astype(BF16)


def _run(heads, orders, start_out):
    chain = []
    for h, order in enumerate(orders):
        for tok in order.split():
            stage, a = tok[0], int(tok[1])
            heads[h + stage.islower()].run(stage.upper(), a, chain)
            if stage in OUT and a == (2 if h else 0):
                start_out(OUT[stage], h)


def _body(*refs):
    hin, hout = refs[:4], refs[4:8]
    ibuf, obuf, robuf, pb0, pb1, ds0, ds1, pbr, dsr, dsc, kc, isem, osem, rsem = refs[8:]
    copy = pltpu.make_async_copy
    iview = lambda b: [b.at[pl.ds(IOFF[t], ILEN[t])] for t in range(4)]
    oview = lambda b: [b.at[pl.ds(OOFF[t], OLEN[t])] for t in range(4)]
    wait = lambda b, sem: copy(b, b, sem).wait()
    carried = lambda slot: _Head([None] * 5 + [oview(slot)[1], None, None], None, dsc, kc)

    def start_head(g, p, j, sem):
        for t in range(4):
            copy(hin[t].at[g], iview(ibuf.at[p, j])[t], sem).start()

    def start_block(n, p):
        for t in range(4):
            copy(hin[t].at[pl.ds(R + n * HB, HB)], ibuf.at[p, :, pl.ds(IOFF[t], ILEN[t])], isem.at[p]).start()

    def ramp_start(h):
        per = -(-HB // R)
        pl.when(h + 1 < R)(lambda: start_head(h + 1, 1, h + 1, rsem.at[(h + 1) & 1]))
        for j in range(per):
            jj = HB - 1 - ((R - 1 - h) * per + j)
            if not isinstance(jj, int):
                pl.when(jnp.logical_and(jj >= 0, jj < HB))(lambda: start_head(R + jj, 0, jj, isem.at[0]))
            elif jj >= 0:
                start_head(R + jj, 0, jj, isem.at[0])

    def zero(i, c):
        dsc[pl.ds(pl.multiple_of(i * 8, 8), 8), :] = jnp.zeros((8, SK), U32)
        return c

    def ramp(h, c):
        head = _Head(iview(ibuf.at[1, h]) + oview(robuf.at[h]), pbr, dsr, kc, dsc)
        _run([carried(robuf.at[h]), head], [PRE, RAMP], lambda t, _: None)
        ramp_start(h + 1)
        pl.when(h + 1 < R)(lambda: wait(ibuf.at[1, h + 1], rsem.at[(h + 1) & 1]))
        return c

    def block(step, c):
        par = step & 1
        heads = [carried(obuf.at[par, HB - 1])]
        for h in range(HB):
            outs = oview(obuf.at[par, h])
            heads.append(_Head(iview(ibuf.at[par, h]) + outs, (pb0, pb1)[h % 2], (ds0, ds1)[h % 2], kc,
                               dsc if h == HB - 1 else None))

        def start_out(t, h):
            if h == 0 or h in GROUPS:
                g = 1 if h == 0 else h - max(e for e in (0,) + GROUPS if e < h)
                lo, n = (0, QB) if h == 0 else (QB, SQ - QB) if (h == HB and t == 1) else (0, OLEN[t])
                copy(obuf.at[par, pl.ds((h - g) % HB, g), pl.ds(OOFF[t] + lo, n)],
                     hout[t].at[pl.ds(R + step * HB + h - g, g), pl.ds(lo, n)], osem.at[par]).start()

        _run(heads, [PRE, FIRST] + [MID] * (HB - 2) + [LAST], start_out)
        pl.when(step + 2 < NSTEPS)(lambda: start_block(step + 2, par))
        pl.when(step >= 1)(lambda: wait(obuf.at[1 - par], osem.at[1 - par]))
        pl.when(step + 1 < NSTEPS)(lambda: wait(ibuf.at[1 - par], isem.at[1 - par]))
        return c

    start_head(0, 1, 0, rsem.at[0])
    lax.fori_loop(0, 8, zero, 0)
    kc[...] = jnp.zeros(kc.shape, U32)
    wait(ibuf.at[1, 0], rsem.at[0])
    ramp_start(0)
    lax.fori_loop(0, R, ramp, 0)
    wait(ibuf.at[0], isem.at[0])
    start_block(1, 1)
    rout = [copy(robuf.at[:, pl.ds(OOFF[t], OLEN[t])], hout[t].at[pl.ds(0, R)], rsem.at[0]) for t in (0, 2, 3)]
    rout.append(copy(robuf.at[pl.ds(1, R - 1), pl.ds(OOFF[1], QB)],
                     hout[1].at[pl.ds(0, R - 1), pl.ds(0, QB)], rsem.at[0]))
    rout.append(copy(robuf.at[:, pl.ds(OOFF[1] + QB, SQ - QB)],
                     hout[1].at[pl.ds(0, R), pl.ds(QB, SQ - QB)], rsem.at[0]))
    for cp in rout:
        cp.start()
    lax.fori_loop(0, NSTEPS, block, 0)
    for cp in rout:
        cp.wait()
    carried(robuf.at[0]).run("Q", 0, [])
    final = copy(robuf.at[0, pl.ds(OOFF[1], QB)], hout[1].at[NH - 1, pl.ds(0, QB)], rsem.at[1])
    final.start()
    wait(obuf.at[(NSTEPS - 1) % 2], osem.at[(NSTEPS - 1) % 2])
    final.wait()


@jax.jit
def pallas_standalone__mha_softmax__near_ridge_kernel(q, k, v, grad_out):
    b, h = q.shape[:2]
    assert (b * h, q.shape[2], k.shape[2], q.shape[3]) == (NH, SQ, SK, D) and R + NSTEPS * HB == NH
    flat = lambda x: x.reshape(NH, x.shape[2], D)
    hbm = pl.BlockSpec(memory_space=pl.ANY)
    slots = pltpu.VMEM((2, HB, ROWS, D), BF16)
    sems = pltpu.SemaphoreType.DMA((2,))
    outs = pl.pallas_call(
        _body,
        in_specs=[hbm] * 4,
        out_specs=[hbm] * 4,
        out_shape=[jax.ShapeDtypeStruct((NH, n, D), BF16) for n in OLEN],
        scratch_shapes=[slots, slots, pltpu.VMEM((R, ROWS, D), BF16)]
        + [pltpu.VMEM((SQ // 2, SK), U32)] * 6
        + [pltpu.VMEM((QB // 2, SK), U32), pltpu.VMEM((SK // 2, D), U32), sems, sems, sems],
        compiler_params=pltpu.CompilerParams(vmem_limit_bytes=120 * 2**20, disable_bounds_checks=True),
        name="mha_fwd_bwd",
    )(flat(q), flat(k), flat(v), flat(grad_out))
    return tuple(o.reshape(b, h, o.shape[1], D) for o in outs)
```
